```python
import os as _os
_os.environ.setdefault("JAX_PLATFORMS", "cpu")
import jax
import jax.numpy as jnp

def _softmax(x, axis=-1):
    return jax.nn.softmax(x, axis=axis)
def _gelu(x):
    return jax.nn.gelu(x, approximate=True)
def _silu(x):
    return jax.nn.silu(x)
def _sigmoid(x):
    return jax.nn.sigmoid(x)
def _layernorm(x, axis=-1, eps=1e-5):
    m = jnp.mean(x, axis=axis, keepdims=True)
    v = jnp.var(x, axis=axis, keepdims=True)
    return (x - m) / jnp.sqrt(v + eps)
def _scatter_add(tgt, idx, src, axis=0):
    return tgt.at[idx].add(src)
def _segment_sum(src, seg, n):
    return jax.ops.segment_sum(src, seg, n)
class _Rng:
    def __init__(self, key):
        self._k = key
    def _next(self):
        self._k, sub = jax.random.split(self._k)
        return sub
    def normal(self, shape):
        return jax.random.normal(self._next(), shape, dtype=jnp.bfloat16)
    def randint(self, lo, hi, shape):
        return jax.random.randint(self._next(), shape, lo, hi, dtype=jnp.int32)
    def uniform(self, shape, lo=0.0, hi=1.0):
        return jax.random.uniform(self._next(), shape, jnp.bfloat16, lo, hi)
    def permutation(self, n):
        return jax.random.permutation(self._next(), n)


kernel_name = 'parallel_sum__grouped_kv_mqa__dense_activation_silu__prompt'

def setup_inputs():
    _rng = _Rng(jax.random.key(int.from_bytes(__import__("os").urandom(4), "little")))
    _w = (lambda a: (lambda t: t.astype(jnp.bfloat16) if jnp.issubdtype(t.dtype, jnp.floating) else t)(jnp.asarray(a)))
    def _A_setup():
        B, S, D, H = 1, 2048, 512, 32
        Dh = D // H
        return {
            "x": _w((lambda *s: _rng.normal(s) * 0.05)(B, S, D)),
            "wq": _w((lambda *s: _rng.normal(s) * 0.05)(D, H * Dh)),
            "wk": _w((lambda *s: _rng.normal(s) * 0.05)(D, Dh)),
            "wv": _w((lambda *s: _rng.normal(s) * 0.05)(D, Dh)),
            "wo": _w((lambda *s: _rng.normal(s) * 0.05)(H * Dh, D)),
        }
    _A_in = _A_setup()

    def _B_setup():
        B, S, D, F = 1, 2048, 512, 1376
        return {
            "x": _w((lambda *s: _rng.normal(s) * 0.05)(B, S, D)),
            "w1": _w((lambda *s: _rng.normal(s) * 0.05)(D, F) * (D ** -0.5)),
            "w2": _w((lambda *s: _rng.normal(s) * 0.05)(F, D) * (F ** -0.5)),
        }
    _B_in = _B_setup()

    return {
        "A_x": _A_in["x"],
        "A_wq": _A_in["wq"],
        "A_wk": _A_in["wk"],
        "A_wv": _A_in["wv"],
        "A_wo": _A_in["wo"],
        "B_x": _B_in["x"],
        "B_w1": _B_in["w1"],
        "B_w2": _B_in["w2"],
    }

def reference(A_x, A_wq, A_wk, A_wv, A_wo, B_x, B_w1, B_w2):
    def _A_ref(x, wq, wk, wv, wo):
        B, S, D = x.shape
        H = 32
        Dh = D // H
        q = (lambda x, *d: x.transpose(*d))((x @ wq).reshape(B, S, H, Dh), 0, 2, 1, 3)
        k = x @ wk
        v = x @ wv
        scores = jnp.einsum("bhqd,bkd->bhqk", q, k) * (Dh ** -0.5)
        p = _softmax(scores, axis=-1)
        o = jnp.einsum("bhqk,bkd->bhqd", p, v)
        return (lambda x, *d: x.transpose(*d))(o, 0, 2, 1, 3).reshape(B, S, H * Dh) @ wo

    def _B_ref(x, w1, w2):
        h = jnp.einsum("bsd,df->bsf", x, w1)
        h = _silu(h)
        out = jnp.einsum("bsf,fd->bsd", h, w2)
        return out

    x = A_x
    xn = _layernorm(x, axis=-1)
    return x + _A_ref(xn, A_wq, A_wk, A_wv, A_wo) + _B_ref(xn, B_w1, B_w2)
```

```python
import math

import jax
import jax.numpy as jnp
from jax import lax
import jax.experimental.pallas as pl
import jax.experimental.pallas.tpu as pltpu

S = 2048
D = 512
H = 32
DH = 16
F = 1376
TQ = 512
NQ = S // TQ
TK = 128
NC = S // TK
T = NQ * H
U = 2
EPS = 1e-5
QSCALE = (DH ** -0.5) * math.log2(math.e)

_NT = (((1,), (1,)), ((), ()))
_TN = (((0,), (0,)), ((), ()))


def _kernel(x_ref, wq_ref, wk_ref, wv_ref, wo_ref, w1_ref, w2_ref, o_ref,
            xn_ref, wT_ref, k_ref, vT_ref, qT_ref, oT_ref, m_ref, *sbufs):
    f32 = jnp.float32
    bf16 = jnp.bfloat16

    wT_ref[0:D, :] = wq_ref[...].astype(f32).T.astype(bf16)
    wT_ref[D:D + DH, :] = wv_ref[...].astype(f32).T.astype(bf16)

    for j in range(NQ):
        rows = slice(j * TQ, (j + 1) * TQ)
        x = x_ref[rows, :].astype(f32)
        mu = jnp.mean(x, axis=-1, keepdims=True)
        xc = x - mu
        var = jnp.mean(xc * xc, axis=-1, keepdims=True)
        xn = (xc * lax.rsqrt(var + EPS)).astype(bf16)
        xn_ref[rows, :] = xn
        r = lax.dot_general(wT_ref[...], xn, _NT, preferred_element_type=f32)
        qT_ref[j * D:(j + 1) * D, :] = (r[0:D] * QSCALE).astype(bf16)
        vT_ref[:, rows] = r[D:D + DH].astype(bf16)
        k_ref[rows, :] = jnp.dot(xn, wk_ref[...],
                                 preferred_element_type=f32).astype(bf16)

    def stage_a(t, sbuf, c, m):
        qh = qT_ref[pl.ds(pl.multiple_of(t * DH, DH), DH), :]
        s = jnp.dot(k_ref[c * TK:(c + 1) * TK, :], qh, preferred_element_type=f32)
        sbuf[c * TK:(c + 1) * TK, :] = s
        mm = jnp.max(s.reshape(TK // 8, 8, TQ), axis=0)
        return mm if m is None else jnp.maximum(m, mm)

    def stage_b(sbuf, c, m, acc, l):
        p = jnp.exp2(sbuf[c * TK:(c + 1) * TK, :] - m)
        o = jnp.dot(vT_ref[:, c * TK:(c + 1) * TK], p.astype(bf16),
                    preferred_element_type=f32)
        for r in reversed(range(TK // 8)):
            pr = p[r * 8:(r + 1) * 8, :]
            l = pr if l is None else l + pr
        return (o if acc is None else acc + o), l

    def step(tb, u, do_a=True, do_b=True):
        sbuf = sbufs[u]
        m_a = acc = l = None
        if do_b:
            m_prev = m_ref[u, 0:1, :]
        for c in range(NC):
            if do_b:
                acc, l = stage_b(sbuf, c, m_prev, acc, l)
            if do_a:
                m_a = stage_a(tb + U, sbuf, c, m_a)
        if do_b:
            lsum = jnp.sum(l, axis=0, keepdims=True)
            oT_ref[pl.ds(pl.multiple_of(tb * DH, DH), DH), :] = (
                acc / lsum).astype(bf16)
        if do_a:
            m_ref[u] = jnp.broadcast_to(
                jnp.max(m_a, axis=0, keepdims=True), (8, TQ))

    for u in range(U):
        step(u - U, u, do_b=False)

    def body(i, carry):
        for u in range(U):
            step(i * U + u, u)
        return carry

    lax.fori_loop(0, T // U - 1, body, 0)
    for u in range(U):
        step(T - U + u, u, do_a=False)

    for j in range(NQ):
        rows = slice(j * TQ, (j + 1) * TQ)
        xn = xn_ref[rows, :]
        h = jnp.dot(xn, w1_ref[...], preferred_element_type=f32)
        h = (h * jax.nn.sigmoid(h)).astype(bf16)
        y = jnp.dot(h, w2_ref[...], preferred_element_type=f32)
        a = lax.dot_general(oT_ref[j * D:(j + 1) * D, :], wo_ref[...], _TN,
                            preferred_element_type=f32)
        o_ref[rows, :] = (x_ref[rows, :].astype(f32) + a + y).astype(o_ref.dtype)


@jax.jit
def pallas_parallel_sum__grouped_kv_mqa__dense_activation_silu__prompt_kernel(
    A_x: jax.Array,
    A_wq: jax.Array,
    A_wk: jax.Array,
    A_wv: jax.Array,
    A_wo: jax.Array,
    B_x: jax.Array,
    B_w1: jax.Array,
    B_w2: jax.Array,
):
    del B_x
    bf16 = jnp.bfloat16
    x2 = A_x.reshape(S, D)
    out = pl.pallas_call(
        _kernel,
        out_shape=jax.ShapeDtypeStruct((S, D), A_x.dtype),
        scratch_shapes=[
            pltpu.VMEM((S, D), bf16),
            pltpu.VMEM((D + DH, D), bf16),
            pltpu.VMEM((S, DH), bf16),
            pltpu.VMEM((DH, S), bf16),
            pltpu.VMEM((NQ * D, TQ), bf16),
            pltpu.VMEM((NQ * D, TQ), bf16),
            pltpu.VMEM((U, 8, TQ), jnp.float32),
        ] + [pltpu.VMEM((S, TQ), jnp.float32) for _ in range(U)],
        compiler_params=pltpu.CompilerParams(
            vmem_limit_bytes=100 * 1024 * 1024),
    )(x2, A_wq, A_wk, A_wv, A_wo, B_w1, B_w2)
    return out.reshape(1, S, D)
```

```python
import math

import jax
import jax.numpy as jnp
from jax import lax
import jax.experimental.pallas as pl
import jax.experimental.pallas.tpu as pltpu

S = 2048
D = 512
H = 32
DH = 16
F = 1376
TQ = 512
NQ = S // TQ
NCT = TQ // 128
TK = 128
NC = S // TK
T = NQ * H
EPS = 1e-5
QSCALE = (DH ** -0.5) * math.log2(math.e)

UF = 4
LAG = 2
NVP = 20
US = 2
SCORE_BOUND = 60.0

_NT = (((1,), (1,)), ((), ()))
_TN = (((0,), (0,)), ((), ()))

_VP = {}
for _i in range(NVP):
    _c4, _j = divmod((_i * 32) // NVP, 8)
    _VP[((_i % 4) * 4 + _c4, _j)] = _i


def _kernel(x_hbm, wq_hbm, wkT_hbm, wvT_hbm, wo_hbm, w1T_hbm, w2_hbm, o_hbm,
            x_ref, wq_ref, wo_ref, w1T_ref, w2_ref, out_ref,
            xn_ref, wT_ref, k_ref, vT_ref, qT_ref, qf_ref, kb_ref, oT_ref,
            m_ref, sb0, sb1, sems):
    f32 = jnp.float32
    bf16 = jnp.bfloat16
    pack = lambda a: pltpu.bitcast(a, jnp.uint32)
    unpack = lambda a: pltpu.bitcast(a, bf16)

    def x_copy(j):
        rows = pl.ds(j * TQ, TQ)
        return pltpu.make_async_copy(x_hbm.at[rows], x_ref.at[rows], sems.at[j])

    cp_wq = pltpu.make_async_copy(wq_hbm, wq_ref, sems.at[NQ])
    cp_wv = pltpu.make_async_copy(wvT_hbm, wT_ref.at[pl.ds(D, DH)], sems.at[NQ + 1])
    cp_wk = pltpu.make_async_copy(wkT_hbm, wT_ref.at[pl.ds(D + DH, DH)],
                                  sems.at[NQ + 2])
    cp_w1 = pltpu.make_async_copy(w1T_hbm, w1T_ref, sems.at[NQ + 3])
    cp_w2 = pltpu.make_async_copy(w2_hbm, w2_ref, sems.at[NQ + 4])
    cp_wo = pltpu.make_async_copy(wo_hbm, wo_ref, sems.at[NQ + 5])

    def out_copy(j):
        rows = pl.ds(j * TQ, TQ)
        return pltpu.make_async_copy(out_ref.at[rows], o_hbm.at[rows],
                                     sems.at[NQ + 6 + j])

    x_copy(0).start()
    cp_wq.start()
    cp_wv.start()
    cp_wk.start()

    def layer_norm(j):
        rows = pl.ds(pl.multiple_of(j * TQ, TQ), TQ)
        x = x_ref[rows, :].astype(f32)
        mu = jnp.mean(x, axis=-1, keepdims=True)
        xc = x - mu
        var = jnp.mean(xc * xc, axis=-1, keepdims=True)
        xn_ref[rows, :] = (xc * lax.rsqrt(var + EPS)).astype(bf16)

    def project(j, xn):
        r = lax.dot_general(wT_ref[...], xn, _NT, preferred_element_type=f32)
        q = (r[0:D] * QSCALE).astype(bf16)
        qT_ref[pl.ds(pl.multiple_of(j * (D // 2), D // 2), D // 2), :] = pack(q)
        qf_ref[pl.ds(j * H, H)] = q.astype(f32).reshape(H, DH, TQ)
        vT_ref[j] = pack(r[D:D + DH].astype(bf16))
        kr = r[D + DH:D + 2 * DH].T.astype(bf16)
        k_ref[pl.ds(pl.multiple_of(j * (TQ // 2), TQ // 2), TQ // 2), :] = pack(kr)
        return jnp.sum((r * r).reshape(H + 2, DH, TQ), axis=1)

    x_copy(0).wait()
    for j in range(1, NQ):
        x_copy(j).start()
    cp_wq.wait()
    cp_wv.wait()
    cp_wk.wait()
    layer_norm(0)
    wT_ref[0:D, :] = wq_ref[...].astype(f32).T.astype(bf16)

    def pro_body(j, n2max):
        x_copy(j + 1).wait()
        xn = xn_ref[pl.ds(pl.multiple_of(j * TQ, TQ), TQ), :]
        layer_norm(j + 1)
        return jnp.maximum(n2max, project(j, xn))

    n2max = lax.fori_loop(0, NQ - 1, pro_body, jnp.zeros((H + 2, TQ), f32))
    cp_w1.start()
    cp_w2.start()
    cp_wo.start()
    n2max = jnp.maximum(n2max, project(NQ - 1, xn_ref[(NQ - 1) * TQ:NQ * TQ, :]))
    for (c, jj), vi in _VP.items():
        k0 = (c * 8 + 7 - jj) * 8
        kf = unpack(k_ref[k0:k0 + 8, :]).astype(f32)
        for d in range(DH):
            kb_ref[vi, d] = jnp.broadcast_to(kf[:, d:d + 1], (16, 128))

    q2 = jnp.max(n2max[0:H]) * (QSCALE * QSCALE)
    v2 = jnp.max(n2max[H:H + 1])
    k2 = jnp.max(n2max[H + 1:H + 2])
    fast = jnp.logical_and(
        q2 * k2 * 1.05 <= SCORE_BOUND * SCORE_BOUND,
        jnp.logical_and(v2 <= 2.0 ** 80, v2 >= 2.0 ** -60))

    def q_tile(t, ct):
        return unpack(qT_ref[pl.ds(pl.multiple_of(t * 8, 8), 8),
                             ct * 128:(ct + 1) * 128])

    def v_tile(c):
        jb, cc = divmod(c, TQ // TK)
        return unpack(vT_ref[jb, :, cc * TK:(cc + 1) * TK])

    def write_o(t, acc, l):
        lsum = jnp.sum(l, axis=0, keepdims=True)
        oT_ref[pl.ds(pl.multiple_of(t * DH, DH), DH), :] = (acc / lsum).astype(bf16)

    @pl.when(fast)
    def _():
        def qk(t, c, ct):
            js = [j for j in range(8) if (c, j) not in _VP]
            kk = jnp.concatenate(
                [k_ref[(c * 8 + 7 - j) * 8:(c * 8 + 8 - j) * 8, :] for j in js],
                axis=0)
            s = jnp.dot(unpack(kk), q_tile(t, ct), preferred_element_type=f32)
            return {j: s[n * 16:(n + 1) * 16] for n, j in enumerate(js)}

        def qk_vpu(t, vi, ct):
            a0 = a1 = None
            for d in range(DH):
                qq = jnp.broadcast_to(
                    qf_ref[t, d:d + 1, ct * 128:(ct + 1) * 128], (8, 128))
                p0 = kb_ref[vi, d, 0:8, :] * qq
                p1 = kb_ref[vi, d, 8:16, :] * qq
                a0 = p0 if a0 is None else a0 + p0
                a1 = p1 if a1 is None else a1 + p1
            return jnp.concatenate([a0, a1], axis=0)

        def pv(t, n, s_m, acc, l):
            pp = [dict() for _ in range(NCT)]
            for j in range(8):
                for ct in range(NCT):
                    c = (n + 4 * ct) % NC
                    sv = qk_vpu(t, _VP[(c, j)], ct) if (c, j) in _VP else s_m[ct][j]
                    p = jnp.exp2(sv)
                    l[ct] = p[0:8] if l[ct] is None else l[ct] + p[0:8]
                    l[ct] = l[ct] + p[8:16]
                    pp[ct][j] = p
            for ct in range(NCT):
                c = (n + 4 * ct) % NC
                pt = jnp.concatenate([pp[ct][j] for j in reversed(range(8))],
                                     axis=0).astype(bf16)
                o = jnp.dot(v_tile(c), pt,
                            preferred_element_type=f32)
                acc[ct] = o if acc[ct] is None else acc[ct] + o
            return acc, l

        def body(i, carry):
            seq = [(u, c) for u in range(UF) for c in range(NC)]
            sm = {}
            st = {u: ([None] * NCT, [None] * NCT) for u in range(UF)}
            for n in range(len(seq) + LAG):
                if n < len(seq):
                    u, c = seq[n]
                    sm[(u, c)] = [qk(i * UF + u, (c + 4 * ct) % NC, ct)
                                  for ct in range(NCT)]
                if n >= LAG:
                    u, c = seq[n - LAG]
                    st[u] = pv(i * UF + u, c, sm.pop((u, c)), *st[u])
                    if c == NC - 1:
                        write_o(i * UF + u, jnp.concatenate(st[u][0], axis=1),
                                jnp.concatenate(st[u][1], axis=1))
            return carry

        lax.fori_loop(0, T // UF, body, 0)

    @pl.when(jnp.logical_not(fast))
    def _():
        sbufs = (sb0, sb1)

        def stage_a(t, sbuf, c, m):
            qh = unpack(qT_ref[pl.ds(pl.multiple_of(t * 8, 8), 8), :])
            s = jnp.dot(unpack(k_ref[c * 64:(c + 1) * 64, :]), qh,
                        preferred_element_type=f32)
            sbuf[c * TK:(c + 1) * TK, :] = s
            mm = jnp.max(s.reshape(TK // 8, 8, TQ), axis=0)
            return mm if m is None else jnp.maximum(m, mm)

        def stage_b(sbuf, c, m, acc, l):
            p = jnp.exp2(sbuf[c * TK:(c + 1) * TK, :] - m)
            o = jnp.dot(v_tile(c), p.astype(bf16),
                        preferred_element_type=f32)
            for r in reversed(range(TK // 8)):
                pr = p[r * 8:(r + 1) * 8, :]
                l = pr if l is None else l + pr
            return (o if acc is None else acc + o), l

        def step(tb, u, do_a=True, do_b=True):
            sbuf = sbufs[u]
            m_a = acc = l = None
            if do_b:
                m_prev = m_ref[u, 0:1, :]
            for c in range(NC):
                if do_b:
                    acc, l = stage_b(sbuf, c, m_prev, acc, l)
                if do_a:
                    m_a = stage_a(tb + US, sbuf, c, m_a)
            if do_b:
                write_o(tb, acc, l)
            if do_a:
                m_ref[u] = jnp.broadcast_to(
                    jnp.max(m_a, axis=0, keepdims=True), (8, TQ))

        for u in range(US):
            step(u - US, u, do_b=False)

        def body(i, carry):
            for u in range(US):
                step(i * US + u, u)
            return carry

        lax.fori_loop(0, T // US - 1, body, 0)
        for u in range(US):
            step(T - US + u, u, do_a=False)

    cp_w1.wait()
    cp_w2.wait()
    cp_wo.wait()
    def epi_body(j, carry):
        rows = pl.ds(pl.multiple_of(j * TQ, TQ), TQ)
        xn = xn_ref[rows, :]
        h = lax.dot_general(xn, w1T_ref[...], _NT, preferred_element_type=f32)
        hh = 0.5 * h
        h = (hh * jnp.tanh(hh) + hh).astype(bf16)
        y = jnp.dot(h, w2_ref[...], preferred_element_type=f32)
        a = lax.dot_general(oT_ref[rows, :], wo_ref[...], _TN,
                            preferred_element_type=f32)
        out_ref[rows, :] = (x_ref[rows, :].astype(f32) + a + y).astype(bf16)
        out_copy(j).start()
        return carry

    lax.fori_loop(0, NQ, epi_body, 0)
    for j in range(NQ):
        out_copy(j).wait()


@jax.jit
def pallas_parallel_sum__grouped_kv_mqa__dense_activation_silu__prompt_kernel(
    A_x: jax.Array,
    A_wq: jax.Array,
    A_wk: jax.Array,
    A_wv: jax.Array,
    A_wo: jax.Array,
    B_x: jax.Array,
    B_w1: jax.Array,
    B_w2: jax.Array,
):
    del B_x
    bf16 = jnp.bfloat16
    f32 = jnp.float32
    u32 = jnp.uint32
    any_spec = pl.BlockSpec(memory_space=pl.ANY)
    out = pl.pallas_call(
        _kernel,
        out_shape=jax.ShapeDtypeStruct((S, D), bf16),
        in_specs=[any_spec] * 7,
        out_specs=any_spec,
        scratch_shapes=[
            pltpu.VMEM((S, D), bf16),
            pltpu.VMEM((D, D), bf16),
            pltpu.VMEM((D, D), bf16),
            pltpu.VMEM((F, D), bf16),
            pltpu.VMEM((F, D), bf16),
            pltpu.VMEM((S, D), bf16),
            pltpu.VMEM((S, D), bf16),
            pltpu.VMEM((D + 2 * DH, D), bf16),
            pltpu.VMEM((S // 2, DH), u32),
            pltpu.VMEM((NQ, DH // 2, TQ), u32),
            pltpu.VMEM((NQ * D // 2, TQ), u32),
            pltpu.VMEM((T, DH, TQ), f32),
            pltpu.VMEM((NVP, DH, 16, 128), f32),
            pltpu.VMEM((NQ * D, TQ), bf16),
            pltpu.VMEM((US, 8, TQ), f32),
            pltpu.VMEM((S, TQ), f32),
            pltpu.VMEM((S, TQ), f32),
            pltpu.SemaphoreType.DMA((2 * NQ + 6,)),
        ],
        compiler_params=pltpu.CompilerParams(
            vmem_limit_bytes=100 * 1024 * 1024),
    )(A_x.reshape(S, D), A_wq, A_wk.T, A_wv.T, A_wo, B_w1.T, B_w2)
    return out.reshape(1, S, D)
```

```python
import math

import jax
import jax.numpy as jnp
from jax import lax
import jax.experimental.pallas as pl
import jax.experimental.pallas.tpu as pltpu

S = 2048
D = 512
H = 32
DH = 16
F = 1376
TQ = 512
NQ = S // TQ
NCT = TQ // 128
TK = 128
NC = S // TK
T = NQ * H
EPS = 1e-5
QSCALE = (DH ** -0.5) * math.log2(math.e)

UF = 8
ROT = 1
LAG = 2
NVP = 16
US = 2
SCORE_BOUND = 60.0

_NT = (((1,), (1,)), ((), ()))
_TN = (((0,), (0,)), ((), ()))

_VP = {}
for _i in range(NVP):
    _c4, _j = divmod((_i * 32) // NVP, 8)
    _VP[((_i % 4) * 4 + _c4, _j)] = _i


def _kernel(x_hbm, wq_hbm, wkT_hbm, wvT_hbm, wo_hbm, w1T_hbm, w2_hbm, o_hbm,
            x_ref, wq_ref, wo_ref, w1T_ref, w2_ref, out_ref,
            xn_ref, wT_ref, k_ref, vT_ref, qT_ref, qf_ref, kb_ref, oT_ref,
            m_ref, sb0, sb1, sc_ref, sems):
    f32 = jnp.float32
    bf16 = jnp.bfloat16
    pack = lambda a: pltpu.bitcast(a, jnp.uint32)
    unpack = lambda a: pltpu.bitcast(a, bf16)

    def x_copy(j):
        rows = pl.ds(j * TQ, TQ)
        return pltpu.make_async_copy(x_hbm.at[rows], x_ref.at[rows], sems.at[j])

    cp_wq = pltpu.make_async_copy(wq_hbm, wq_ref, sems.at[NQ])
    cp_wv = pltpu.make_async_copy(wvT_hbm, wT_ref.at[pl.ds(DH, DH)], sems.at[NQ + 1])
    cp_wk = pltpu.make_async_copy(wkT_hbm, wT_ref.at[pl.ds(0, DH)],
                                  sems.at[NQ + 2])
    cp_w1 = pltpu.make_async_copy(w1T_hbm, w1T_ref, sems.at[NQ + 3])
    cp_w2 = pltpu.make_async_copy(w2_hbm, w2_ref, sems.at[NQ + 4])
    cp_wo = pltpu.make_async_copy(wo_hbm, wo_ref, sems.at[NQ + 5])

    def out_copy(j):
        rows = pl.ds(j * TQ, TQ)
        return pltpu.make_async_copy(out_ref.at[rows], o_hbm.at[rows],
                                     sems.at[NQ + 6 + j])

    x_copy(0).start()
    cp_wq.start()
    cp_wv.start()
    cp_wk.start()

    def layer_norm(j):
        rows = slice(j * TQ, (j + 1) * TQ)
        x = x_ref[rows, :].astype(f32)
        mu = jnp.mean(x, axis=-1, keepdims=True)
        xc = x - mu
        var = jnp.mean(xc * xc, axis=-1, keepdims=True)
        xn = (xc * lax.rsqrt(var + EPS)).astype(bf16)
        xn_ref[rows, :] = xn
        return xn

    def project(j, xn):
        r = lax.dot_general(wT_ref[...], xn, _NT, preferred_element_type=f32)
        kr = r[0:DH].T.astype(bf16)
        k_ref[j * (TQ // 2):(j + 1) * (TQ // 2), :] = pack(kr)
        kf = kr.astype(f32)
        for (c, jj), vi in _VP.items():
            k0 = (c * 8 + 7 - jj) * 16 - j * TQ
            if 0 <= k0 < TQ:
                for d in range(DH):
                    kb_ref[vi, d] = jnp.broadcast_to(
                        kf[k0:k0 + 16, d:d + 1], (16, 128))
        vT_ref[j] = pack(r[DH:2 * DH].astype(bf16))
        q = (r[2 * DH:] * QSCALE).astype(bf16)
        qT_ref[j * (D // 2):(j + 1) * (D // 2), :] = pack(q)
        qf_ref[j * H:(j + 1) * H] = q.astype(f32).reshape(H, DH, TQ)
        n2 = jnp.sum((r * r).reshape(H + 2, DH, TQ), axis=1)
        return (n2[0:1], n2[1:2], jnp.max(n2[2:], axis=0, keepdims=True))

    x_copy(0).wait()
    for j in range(1, NQ):
        x_copy(j).start()
    cp_wq.wait()
    cp_wv.wait()
    cp_wk.wait()
    wT_ref[2 * DH:, :] = wq_ref[...].astype(f32).T.astype(bf16)
    n2 = project(0, layer_norm(0))
    for j in range(1, NQ):
        x_copy(j).wait()
    cp_w1.start()
    cp_w2.start()
    cp_wo.start()
    for j in range(1, NQ):
        n2 = tuple(jnp.maximum(a, b) for a, b in zip(n2, project(j, layer_norm(j))))

    k2 = jnp.max(n2[0])
    v2 = jnp.max(n2[1])
    q2 = jnp.max(n2[2]) * (QSCALE * QSCALE)
    fast = jnp.logical_and(
        q2 * k2 * 1.05 <= SCORE_BOUND * SCORE_BOUND,
        jnp.logical_and(v2 <= 2.0 ** 80, v2 >= 2.0 ** -60))

    def q_tile(t, ct):
        return unpack(qT_ref[pl.ds(pl.multiple_of(t * 8, 8), 8),
                             ct * 128:(ct + 1) * 128])

    def v_tile(c):
        jb, cc = divmod(c, TQ // TK)
        return unpack(vT_ref[jb, :, cc * TK:(cc + 1) * TK])

    def write_o(t, acc, l):
        lsum = jnp.sum(l, axis=0, keepdims=True)
        oT_ref[pl.ds(pl.multiple_of(t * DH, DH), DH), :] = (acc / lsum).astype(bf16)

    @pl.when(fast)
    def _():
        def qk(t, c, ct):
            js = [j for j in range(8) if (c, j) not in _VP]
            kk = jnp.concatenate(
                [k_ref[(c * 8 + 7 - j) * 8:(c * 8 + 8 - j) * 8, :] for j in js],
                axis=0)
            s = jnp.dot(unpack(kk), q_tile(t, ct), preferred_element_type=f32)
            return {j: s[n * 16:(n + 1) * 16] for n, j in enumerate(js)}

        def qk_vpu(t, vi, ct):
            a0 = a1 = None
            for d in range(DH):
                qq = jnp.broadcast_to(
                    qf_ref[t, d:d + 1, ct * 128:(ct + 1) * 128], (8, 128))
                p0 = kb_ref[vi, d, 0:8, :] * qq
                p1 = kb_ref[vi, d, 8:16, :] * qq
                a0 = p0 if a0 is None else a0 + p0
                a1 = p1 if a1 is None else a1 + p1
            return jnp.concatenate([a0, a1], axis=0)

        def pv(t, n, s_m, acc, l):
            pp = [dict() for _ in range(NCT)]
            for j in range(8):
                for ct in range(NCT):
                    c = (n + 4 * ct) % NC
                    sv = qk_vpu(t, _VP[(c, j)], ct) if (c, j) in _VP else s_m[ct][j]
                    p = jnp.exp2(sv)
                    l[ct] = p[0:8] if l[ct] is None else l[ct] + p[0:8]
                    l[ct] = l[ct] + p[8:16]
                    pp[ct][j] = p
            for ct in range(NCT):
                c = (n + 4 * ct) % NC
                pt = jnp.concatenate([pp[ct][j] for j in reversed(range(8))],
                                     axis=0).astype(bf16)
                o = jnp.dot(v_tile(c), pt,
                            preferred_element_type=f32)
                acc[ct] = o if acc[ct] is None else acc[ct] + o
            return acc, l

        def qk_all(t, c):
            return [qk(t, (c + 4 * ct) % NC, ct) for ct in range(NCT)]

        def stash(c, s):
            for ct in range(NCT):
                for j, v in s[ct].items():
                    sc_ref[c, ct, j] = v

        def unstash(c):
            return [{j: sc_ref[c, ct, j] for j in range(8)
                     if ((c + 4 * ct) % NC, j) not in _VP} for ct in range(NCT)]

        def body(i, carry):
            seq = [(u, c) for u in range(UF) for c in range(NC)]
            sm = {}
            st = {u: ([None] * NCT, [None] * NCT) for u in range(UF)}
            t_next = jnp.minimum((i + 1) * UF, T - 1)
            for n in range(len(seq) + LAG):
                if n < len(seq):
                    u, c = seq[n]
                    if n < ROT:
                        sm[(u, c)] = unstash(n)
                    else:
                        sm[(u, c)] = qk_all(i * UF + u, c)
                elif n - len(seq) < ROT:
                    stash(n - len(seq), qk_all(t_next, n - len(seq)))
                if n >= LAG:
                    u, c = seq[n - LAG]
                    st[u] = pv(i * UF + u, c, sm.pop((u, c)), *st[u])
                    if c == NC - 1:
                        write_o(i * UF + u, jnp.concatenate(st[u][0], axis=1),
                                jnp.concatenate(st[u][1], axis=1))
            return carry

        if ROT:
            for n in range(ROT):
                stash(n, qk_all(0, n))
        lax.fori_loop(0, T // UF, body, 0)

    @pl.when(jnp.logical_not(fast))
    def _():
        sbufs = (sb0, sb1)

        def stage_a(t, sbuf, c, m):
            qh = unpack(qT_ref[pl.ds(pl.multiple_of(t * 8, 8), 8), :])
            s = jnp.dot(unpack(k_ref[c * 64:(c + 1) * 64, :]), qh,
                        preferred_element_type=f32)
            sbuf[c * TK:(c + 1) * TK, :] = s
            mm = jnp.max(s.reshape(TK // 8, 8, TQ), axis=0)
            return mm if m is None else jnp.maximum(m, mm)

        def stage_b(sbuf, c, m, acc, l):
            p = jnp.exp2(sbuf[c * TK:(c + 1) * TK, :] - m)
            o = jnp.dot(v_tile(c), p.astype(bf16),
                        preferred_element_type=f32)
            for r in reversed(range(TK // 8)):
                pr = p[r * 8:(r + 1) * 8, :]
                l = pr if l is None else l + pr
            return (o if acc is None else acc + o), l

        def step(tb, u, do_a=True, do_b=True):
            sbuf = sbufs[u]
            m_a = acc = l = None
            if do_b:
                m_prev = m_ref[u, 0:1, :]
            for c in range(NC):
                if do_b:
                    acc, l = stage_b(sbuf, c, m_prev, acc, l)
                if do_a:
                    m_a = stage_a(tb + US, sbuf, c, m_a)
            if do_b:
                write_o(tb, acc, l)
            if do_a:
                m_ref[u] = jnp.broadcast_to(
                    jnp.max(m_a, axis=0, keepdims=True), (8, TQ))

        for u in range(US):
            step(u - US, u, do_b=False)

        def body(i, carry):
            for u in range(US):
                step(i * US + u, u)
            return carry

        lax.fori_loop(0, T // US - 1, body, 0)
        for u in range(US):
            step(T - US + u, u, do_a=False)

    cp_w1.wait()
    cp_w2.wait()
    cp_wo.wait()
    def epi_body(j, carry):
        rows = pl.ds(pl.multiple_of(j * TQ, TQ), TQ)
        xn = xn_ref[rows, :]
        h = lax.dot_general(xn, w1T_ref[...], _NT, preferred_element_type=f32)
        hh = 0.5 * h
        h = (hh * jnp.tanh(hh) + hh).astype(bf16)
        y = jnp.dot(h, w2_ref[...], preferred_element_type=f32)
        a = lax.dot_general(oT_ref[rows, :], wo_ref[...], _TN,
                            preferred_element_type=f32)
        out_ref[rows, :] = (x_ref[rows, :].astype(f32) + a + y).astype(bf16)
        out_copy(j).start()
        return carry

    lax.fori_loop(0, NQ, epi_body, 0)
    for j in range(NQ):
        out_copy(j).wait()


@jax.jit
def pallas_parallel_sum__grouped_kv_mqa__dense_activation_silu__prompt_kernel(
    A_x: jax.Array,
    A_wq: jax.Array,
    A_wk: jax.Array,
    A_wv: jax.Array,
    A_wo: jax.Array,
    B_x: jax.Array,
    B_w1: jax.Array,
    B_w2: jax.Array,
):
    del B_x
    bf16 = jnp.bfloat16
    f32 = jnp.float32
    u32 = jnp.uint32
    any_spec = pl.BlockSpec(memory_space=pl.ANY)
    out = pl.pallas_call(
        _kernel,
        out_shape=jax.ShapeDtypeStruct((S, D), bf16),
        in_specs=[any_spec] * 7,
        out_specs=any_spec,
        scratch_shapes=[
            pltpu.VMEM((S, D), bf16),
            pltpu.VMEM((D, D), bf16),
            pltpu.VMEM((D, D), bf16),
            pltpu.VMEM((F, D), bf16),
            pltpu.VMEM((F, D), bf16),
            pltpu.VMEM((S, D), bf16),
            pltpu.VMEM((S, D), bf16),
            pltpu.VMEM((D + 2 * DH, D), bf16),
            pltpu.VMEM((S // 2, DH), u32),
            pltpu.VMEM((NQ, DH // 2, TQ), u32),
            pltpu.VMEM((NQ * D // 2, TQ), u32),
            pltpu.VMEM((T, DH, TQ), f32),
            pltpu.VMEM((NVP, DH, 16, 128), f32),
            pltpu.VMEM((NQ * D, TQ), bf16),
            pltpu.VMEM((US, 8, TQ), f32),
            pltpu.VMEM((S, TQ), f32),
            pltpu.VMEM((S, TQ), f32),
            pltpu.VMEM((ROT, NCT, 8, 16, 128), f32),
            pltpu.SemaphoreType.DMA((2 * NQ + 6,)),
        ],
        compiler_params=pltpu.CompilerParams(
            vmem_limit_bytes=100 * 1024 * 1024),
    )(A_x.reshape(S, D), A_wq, A_wk.T, A_wv.T, A_wo, B_w1.T, B_w2)
    return out.reshape(1, S, D)
```

```python
import math

import jax
import jax.numpy as jnp
from jax import lax
import jax.experimental.pallas as pl
import jax.experimental.pallas.tpu as pltpu

S = 2048
D = 512
H = 32
DH = 16
F = 1376
TQ = 512
NQ = S // TQ
NCT = TQ // 128
TK = 128
NC = S // TK
T = NQ * H
NFT = -(-F // 128)
EPS = 1e-5
QSCALE = (DH ** -0.5) * math.log2(math.e)
SCORE_BOUND = 60.0

UF = 8
NREG = 13
SP = T - UF * NREG
FS = SP // NQ
LAG = 2
UG = 4
POS_A = (0, 2, 4, 6)
POS_B = (4, 6, 0, 2)
OUT_CUTS = (0, 512, 1024, 1536, 1792, 1920, 2048)

_NT = (((1,), (1,)), ((), ()))
_TN = (((0,), (0,)), ((), ()))


def _mxu_groups(c, special):
    skip = (POS_A[c // 4], POS_B[c // 4]) if special else (POS_A[c // 4],)
    return [j for j in range(8) if j not in skip]


def _kernel(x_hbm, wq_hbm, wkT_hbm, wvT_hbm, wo_hbm, w1T_hbm, w2_hbm, o_hbm,
            x_ref, wq_ref, wo_ref, w1T_ref, w2_ref, out_ref,
            xn_ref, wT_ref, km_ref, vT_ref, qT_ref, qf_ref, kba_ref, kbb_ref,
            oT_ref, xy_ref, sv_ref, sc_ref, m_ref, sbuf, sems):
    f32 = jnp.float32
    bf16 = jnp.bfloat16
    pack = lambda a: pltpu.bitcast(a, jnp.uint32)
    unpack = lambda a: pltpu.bitcast(a, bf16)

    def x_copy(j):
        rows = pl.ds(j * TQ, TQ)
        return pltpu.make_async_copy(x_hbm.at[rows], x_ref.at[rows], sems.at[j])

    cp_wq = pltpu.make_async_copy(wq_hbm, wq_ref, sems.at[NQ])
    cp_wk = pltpu.make_async_copy(wkT_hbm, wT_ref.at[pl.ds(0, DH)], sems.at[NQ + 1])
    cp_wv = pltpu.make_async_copy(wvT_hbm, wT_ref.at[pl.ds(DH, DH)], sems.at[NQ + 2])
    cp_w1 = pltpu.make_async_copy(w1T_hbm, w1T_ref, sems.at[NQ + 3])
    cp_w2 = pltpu.make_async_copy(w2_hbm, w2_ref, sems.at[NQ + 4])
    cp_wo = pltpu.make_async_copy(wo_hbm, wo_ref, sems.at[NQ + 5])

    def out_copy(k):
        rows = pl.ds(OUT_CUTS[k], OUT_CUTS[k + 1] - OUT_CUTS[k])
        return pltpu.make_async_copy(out_ref.at[rows], o_hbm.at[rows],
                                     sems.at[NQ + 6 + k])

    x_copy(0).start()
    cp_wq.start()
    cp_wk.start()
    cp_wv.start()

    def layer_norm(j):
        rows = slice(j * TQ, (j + 1) * TQ)
        x = x_ref[rows, :].astype(f32)
        mu = jnp.mean(x, axis=-1, keepdims=True)
        xc = x - mu
        var = jnp.mean(xc * xc, axis=-1, keepdims=True)
        xn = (xc * lax.rsqrt(var + EPS)).astype(bf16)
        xn_ref[rows, :] = xn
        return xn

    def project(j, xn):
        r = lax.dot_general(wT_ref[...], xn, _NT, preferred_element_type=f32)
        kr = r[0:DH].T.astype(bf16)
        kp = pack(kr)
        kf = kr.astype(f32)
        for cc in range(TQ // TK):
            c = j * (TQ // TK) + cc
            km_ref[0, c] = kp[cc * 64:(cc + 1) * 64]
            for v, special in ((1, False), (2, True)):
                js = _mxu_groups(c, special)
                km_ref[v, c, 0:8 * len(js), :] = jnp.concatenate(
                    [kp[(cc * 8 + 7 - jj) * 8:(cc * 8 + 8 - jj) * 8] for jj in js],
                    axis=0)
            k0 = (cc * 8 + 7 - POS_B[j]) * 16
            for d in range(DH):
                kbb_ref[c, d] = jnp.broadcast_to(kf[k0:k0 + 16, d:d + 1], (16, 128))
        vT_ref[j] = pack(r[DH:2 * DH].astype(bf16))
        q = (r[2 * DH:] * QSCALE).astype(bf16)
        qT_ref[j * (D // 2):(j + 1) * (D // 2), :] = pack(q)
        qf_ref[j * H:(j + 1) * H] = q.astype(f32).reshape(H, DH, TQ)
        n2 = jnp.sum((r * r).reshape(H + 2, DH, TQ), axis=1)
        return (n2[0:1], n2[1:2], jnp.max(n2[2:], axis=0, keepdims=True))

    x_copy(0).wait()
    for j in range(1, NQ):
        x_copy(j).start()
    cp_wq.wait()
    cp_wk.wait()
    cp_wv.wait()
    wT_ref[2 * DH:, :] = wq_ref[...].astype(f32).T.astype(bf16)
    n2 = project(0, layer_norm(0))
    for j in range(1, NQ):
        x_copy(j).wait()
    cp_w1.start()
    cp_w2.start()
    for j in range(1, NQ):
        n2 = tuple(jnp.maximum(a, b) for a, b in zip(n2, project(j, layer_norm(j))))

    k2 = jnp.max(n2[0])
    v2 = jnp.max(n2[1])
    q2 = jnp.max(n2[2]) * (QSCALE * QSCALE)
    fast = jnp.logical_and(
        q2 * k2 * 1.05 <= SCORE_BOUND * SCORE_BOUND,
        jnp.logical_and(v2 <= 2.0 ** 80, v2 >= 2.0 ** -60))
    never = q2 < -1.0

    def q_tile(t, ct):
        return unpack(qT_ref[pl.ds(pl.multiple_of(t * 8, 8), 8),
                             ct * 128:(ct + 1) * 128])

    def v_tile(c):
        jb, cc = divmod(c, TQ // TK)
        return unpack(vT_ref[jb, :, cc * TK:(cc + 1) * TK])

    def write_o(t, acc, l):
        lsum = jnp.sum(l, axis=0, keepdims=True)
        oT_ref[pl.ds(pl.multiple_of(t * DH, DH), DH), :] = (acc / lsum).astype(bf16)

    def q_rows(t, ct, first=False):
        rows = [jnp.broadcast_to(qf_ref[t, d:d + 1, ct * 128:(ct + 1) * 128],
                                 (16, 128)) for d in range(DH)]
        cuts = ([0, 1] if first else [0]) + list(range(UG, DH + 1, UG))
        return [(a, b, jnp.stack(rows[a:b])) for a, b in zip(cuts, cuts[1:])]

    def vpu_scores(kb, qb, trigger=None):
        sv = None
        for a, b, q in qb:
            pr = kb[a:b] * q
            if sv is not None:
                pr = jnp.concatenate([sv, pr], axis=0)
            if sv is None and trigger is not None:
                sv = jnp.where(never, trigger[None], pr)
            else:
                sv = jnp.sum(pr, axis=0, keepdims=True)
        return sv[0]

    cp_w1.wait()
    cp_w2.wait()
    cp_wo.start()

    def ffn_body(j, carry):
        rows = pl.ds(pl.multiple_of(j * TQ, TQ), TQ)
        xn = xn_ref[rows, :]
        pos = sum(jnp.where(j == jq, 7 - POS_A[jq], 0) for jq in range(NQ))
        for cc in range(TQ // TK):
            c = j * (TQ // TK) + cc
            kf = unpack(km_ref[0, c, pl.ds(pl.multiple_of(pos * 8, 8), 8), :]
                        ).astype(f32)
            for d in range(DH):
                kba_ref[c, d] = jnp.broadcast_to(kf[:, d:d + 1], (16, 128))

        nunits, njobs = FS * NC * NCT, 2 * NFT - 1
        per = -(-nunits // njobs)
        state = dict(done=0, job=0, qb=None)

        def hosted(res):
            for k in range(per):
                r0 = (k * TQ // per) // 16 * 16
                upto = (state["job"] * per + k + 1) * nunits // (njobs * per)
                while state["done"] < upto:
                    ks, rem = divmod(state["done"], NC * NCT)
                    ct, c = divmod(rem, NC)
                    if c == 0:
                        state["qb"] = q_rows(T - SP + j * FS + ks, ct, first=True)
                    sv_ref[j * FS + ks, c, ct] = vpu_scores(
                        kbb_ref.at[c], state["qb"], res[r0:r0 + 16, 0:128])
                    state["done"] += 1
            state["job"] += 1

        def up(n):
            h = lax.dot_general(xn, w1T_ref[n * 128:min((n + 1) * 128, F), :], _NT,
                                preferred_element_type=f32)
            if n < NFT - 1:
                hosted(h)
            hh = 0.5 * h
            return (hh * jnp.tanh(hh) + hh).astype(bf16)

        def down(g, n):
            y = jnp.dot(g, w2_ref[n * 128:min((n + 1) * 128, F), :],
                        preferred_element_type=f32)
            hosted(y)
            return y

        y = x_ref[rows, :].astype(f32)
        g = up(0)
        for n in range(NFT):
            gn = up(n + 1) if n + 1 < NFT else None
            y = y + down(g, n)
            g = gn
        xy_ref[rows, :] = y
        return carry

    lax.fori_loop(0, NQ, ffn_body, 0)

    @pl.when(fast)
    def _():
        def qk(t, n, special):
            out = []
            for ct in range(NCT):
                c = (n + 4 * ct) % NC
                kk = km_ref[2 if special else 1, c,
                            0:8 * len(_mxu_groups(c, special)), :]
                out.append(jnp.dot(unpack(kk), q_tile(t, ct),
                                   preferred_element_type=f32))
            return out

        def pv(n, s_m, qb, acc, l, s):
            ps = []
            for ct in range(NCT):
                c = (n + 4 * ct) % NC
                js = _mxu_groups(c, s is not None)
                parts, r0 = [], 0
                for j in range(8):
                    if j in js:
                        continue
                    r1 = 16 * len([jj for jj in js if jj < j])
                    if r1 > r0:
                        parts.append(s_m[ct][r0:r1])
                    r0 = r1
                    if j == POS_A[c // 4]:
                        parts.append(vpu_scores(kba_ref.at[c], qb[ct]))
                    else:
                        parts.append(sv_ref[s, c, ct])
                if r0 < 16 * len(js):
                    parts.append(s_m[ct][r0:])
                ps.append(jnp.concatenate(parts, axis=0))
            pw = jnp.exp2(jnp.concatenate(ps, axis=1))
            if l is not None:
                l = jnp.sum(jnp.concatenate([l, pw], axis=0).reshape(
                    TK // 8 + 1, 8, TQ), axis=0)
            else:
                l = jnp.sum(pw.reshape(TK // 8, 8, TQ), axis=0)
            pw = jnp.concatenate(
                [pw[j * 16:(j + 1) * 16] for j in reversed(range(8))], axis=0)
            for ct in range(NCT):
                o = jnp.dot(v_tile((n + 4 * ct) % NC),
                            pw[:, ct * 128:(ct + 1) * 128].astype(bf16),
                            preferred_element_type=f32)
                acc[ct] = o if acc[ct] is None else acc[ct] + o
            return acc, l

        def stash(s):
            for ct in range(NCT):
                sc_ref[ct] = s[ct]

        def make_body(t_base, special):
            def body(i, carry):
                nslots = UF * NC
                t0 = t_base + i * UF
                t_next = jnp.minimum(t0 + UF, T - 1)
                full = {0: [sc_ref[ct] for ct in range(NCT)]}
                for m in range(1, nslots + LAG):
                    if m < nslots:
                        full[m] = qk(t0 + m // NC, m % NC, special)
                    elif m == nslots:
                        stash(qk(t_next, 0, False))
                    n = m - LAG
                    if n >= 0:
                        u, c = divmod(n, NC)
                        if c == 0:
                            if u == 0:
                                acc, l = [None] * NCT, None
                            else:
                                acc, l = [a * 0.0 for a in acc], l * 0.0
                            qb = [q_rows(t0 + u, ct) for ct in range(NCT)]
                        s = i * UF + u if special and n > 0 else None
                        acc, l = pv(c, full.pop(n), qb, acc, l, s)
                        if c == NC - 1:
                            write_o(t0 + u, jnp.concatenate(acc, axis=1), l)
                return carry
            return body

        stash(qk(0, 0, False))
        lax.fori_loop(0, NREG, make_body(0, False), 0)
        lax.fori_loop(0, SP // UF, make_body(T - SP, True), 0)

    @pl.when(jnp.logical_not(fast))
    def _():
        def stage_a(t, c, m):
            qh = unpack(qT_ref[pl.ds(pl.multiple_of(t * 8, 8), 8), :])
            s = jnp.dot(unpack(km_ref[0, c]), qh, preferred_element_type=f32)
            sbuf[c * TK:(c + 1) * TK, :] = s
            mm = jnp.max(s.reshape(TK // 8, 8, TQ), axis=0)
            return mm if m is None else jnp.maximum(m, mm)

        def stage_b(c, m, acc, l):
            p = jnp.exp2(sbuf[c * TK:(c + 1) * TK, :] - m)
            o = jnp.dot(v_tile(c), p.astype(bf16), preferred_element_type=f32)
            for r in reversed(range(TK // 8)):
                pr = p[r * 8:(r + 1) * 8, :]
                l = pr if l is None else l + pr
            return (o if acc is None else acc + o), l

        def step(tb, do_b=True):
            m_a = acc = l = None
            if do_b:
                m_prev = m_ref[0:1, :]
            ta = jnp.minimum(tb + 1, T - 1)
            for c in range(NC):
                if do_b:
                    acc, l = stage_b(c, m_prev, acc, l)
                m_a = stage_a(ta, c, m_a)
            if do_b:
                write_o(tb, acc, l)
            m_ref[...] = jnp.broadcast_to(
                jnp.max(m_a, axis=0, keepdims=True), (8, TQ))

        step(-1, do_b=False)

        def body(t, carry):
            step(t)
            return carry

        lax.fori_loop(0, T, body, 0)

    cp_wo.wait()
    for k in range(len(OUT_CUTS) - 1):
        r0, r1 = OUT_CUTS[k], OUT_CUTS[k + 1]
        j = r0 // TQ
        a = lax.dot_general(oT_ref[j * D:(j + 1) * D, r0 - j * TQ:r1 - j * TQ],
                            wo_ref[...], _TN, preferred_element_type=f32)
        out_ref[r0:r1, :] = (xy_ref[r0:r1, :] + a).astype(bf16)
        out_copy(k).start()
    for k in range(len(OUT_CUTS) - 1):
        out_copy(k).wait()


@jax.jit
def pallas_parallel_sum__grouped_kv_mqa__dense_activation_silu__prompt_kernel(
    A_x: jax.Array,
    A_wq: jax.Array,
    A_wk: jax.Array,
    A_wv: jax.Array,
    A_wo: jax.Array,
    B_x: jax.Array,
    B_w1: jax.Array,
    B_w2: jax.Array,
):
    del B_x
    bf16 = jnp.bfloat16
    f32 = jnp.float32
    u32 = jnp.uint32
    any_spec = pl.BlockSpec(memory_space=pl.ANY)
    out = pl.pallas_call(
        _kernel,
        out_shape=jax.ShapeDtypeStruct((S, D), bf16),
        in_specs=[any_spec] * 7,
        out_specs=any_spec,
        scratch_shapes=[
            pltpu.VMEM((S, D), bf16),
            pltpu.VMEM((D, D), bf16),
            pltpu.VMEM((D, D), bf16),
            pltpu.VMEM((F, D), bf16),
            pltpu.VMEM((F, D), bf16),
            pltpu.VMEM((S, D), bf16),
            pltpu.VMEM((S, D), bf16),
            pltpu.VMEM((D + 2 * DH, D), bf16),
            pltpu.VMEM((3, NC, TK // 2, DH), u32),
            pltpu.VMEM((NQ, DH // 2, TQ), u32),
            pltpu.VMEM((NQ * D // 2, TQ), u32),
            pltpu.VMEM((T, DH, TQ), f32),
            pltpu.VMEM((NC, DH, 16, 128), f32),
            pltpu.VMEM((NC, DH, 16, 128), f32),
            pltpu.VMEM((NQ * D, TQ), bf16),
            pltpu.VMEM((S, D), f32),
            pltpu.VMEM((SP, NC, NCT, 16, 128), f32),
            pltpu.VMEM((NCT, TK - 16, 128), f32),
            pltpu.VMEM((8, TQ), f32),
            pltpu.VMEM((S, TQ), f32),
            pltpu.SemaphoreType.DMA((NQ + 6 + len(OUT_CUTS) - 1,)),
        ],
        compiler_params=pltpu.CompilerParams(
            vmem_limit_bytes=100 * 1024 * 1024),
    )(A_x.reshape(S, D), A_wq, A_wk.T, A_wv.T, A_wo, B_w1.T, B_w2)
    return out.reshape(1, S, D)
```

```python
import math

import jax
import jax.numpy as jnp
from jax import lax
import jax.experimental.pallas as pl
import jax.experimental.pallas.tpu as pltpu

S = 2048
D = 512
H = 32
DH = 16
F = 1376
TQ = 512
NQ = S // TQ
NCT = TQ // 128
TK = 128
NC = S // TK
T = NQ * H
NFT = -(-F // 128)
EPS = 1e-5
QSCALE = (DH ** -0.5) * math.log2(math.e)
SCORE_BOUND = 60.0

UF = 8
NREG = 12
SP = T - UF * NREG
FS = 7
OS = SP - NQ * FS
NEARLY = 3
LAG = 2
UG = 4
POS_A = (0, 2, 4, 6)
POS_B = (4, 4, 0, 0)
OUT_CUTS = (0, 512, 1024, 1536, 1792, 1920, 2048)

_NT = (((1,), (1,)), ((), ()))
_TN = (((0,), (0,)), ((), ()))


def _mxu_groups(c, special):
    skip = (POS_A[c // 4], POS_B[c // 4]) if special else (POS_A[c // 4],)
    return [j for j in range(8) if j not in skip]


def _kernel(x_hbm, wq_hbm, wkT_hbm, wvT_hbm, wo_hbm, w1T_hbm, w2_hbm, o_hbm,
            x_ref, wq_ref, wo_ref, w1T_ref, w2_ref, out_ref,
            xn_ref, wT_ref, km_ref, vT_ref, qT_ref, qf_ref, kba_ref, kbb_ref,
            oT_ref, xy_ref, sv_ref, sc_ref, sbuf, sems):
    f32 = jnp.float32
    bf16 = jnp.bfloat16
    pack = lambda a: pltpu.bitcast(a, jnp.uint32)
    unpack = lambda a: pltpu.bitcast(a, bf16)

    def x_copy(j):
        rows = pl.ds(j * TQ, TQ)
        return pltpu.make_async_copy(x_hbm.at[rows], x_ref.at[rows], sems.at[j])

    cp_wq = pltpu.make_async_copy(wq_hbm, wq_ref, sems.at[NQ])
    cp_wk = pltpu.make_async_copy(wkT_hbm, wT_ref.at[pl.ds(0, DH)], sems.at[NQ + 1])
    cp_wv = pltpu.make_async_copy(wvT_hbm, wT_ref.at[pl.ds(DH, DH)], sems.at[NQ + 2])
    cp_w1 = pltpu.make_async_copy(w1T_hbm, w1T_ref, sems.at[NQ + 3])
    cp_w2 = pltpu.make_async_copy(w2_hbm, w2_ref, sems.at[NQ + 4])
    cp_wo = pltpu.make_async_copy(wo_hbm, wo_ref, sems.at[NQ + 5])

    def out_copy(k):
        rows = pl.ds(OUT_CUTS[k], OUT_CUTS[k + 1] - OUT_CUTS[k])
        return pltpu.make_async_copy(out_ref.at[rows], o_hbm.at[rows],
                                     sems.at[NQ + 6 + k])

    x_copy(0).start()
    cp_wq.start()
    cp_wk.start()
    cp_wv.start()

    def layer_norm(j):
        rows = slice(j * TQ, (j + 1) * TQ)
        x = x_ref[rows, :].astype(f32)
        mu = jnp.mean(x, axis=-1, keepdims=True)
        xc = x - mu
        var = jnp.mean(xc * xc, axis=-1, keepdims=True)
        xn = (xc * lax.rsqrt(var + EPS)).astype(bf16)
        xn_ref[rows, :] = xn
        return xn

    def project(j, xn):
        r = lax.dot_general(wT_ref[...], xn, _NT, preferred_element_type=f32)
        kr = r[0:DH].T.astype(bf16)
        kp = pack(kr)
        kf = kr.astype(f32)
        for cc in range(TQ // TK):
            c = j * (TQ // TK) + cc
            km_ref[0, c] = kp[cc * 64:(cc + 1) * 64]
            for v, special in ((1, False), (2, True)):
                js = _mxu_groups(c, special)
                km_ref[v, c, 0:8 * len(js), :] = jnp.concatenate(
                    [kp[(cc * 8 + 7 - jj) * 8:(cc * 8 + 8 - jj) * 8] for jj in js],
                    axis=0)
            k0 = (cc * 8 + 7 - POS_B[j]) * 16
            for d in range(DH):
                kbb_ref[c, d] = jnp.broadcast_to(kf[k0:k0 + 16, d:d + 1], (16, 128))
        vT_ref[j] = pack(r[DH:2 * DH].astype(bf16))
        q = (r[2 * DH:] * QSCALE).astype(bf16)
        qT_ref[j * (D // 2):(j + 1) * (D // 2), :] = pack(q)
        qf_ref[j * H:(j + 1) * H] = q.astype(f32).reshape(H, DH, TQ)
        n2 = jnp.sum((r * r).reshape(H + 2, DH, TQ), axis=1)
        return (n2[0:1], n2[1:2], jnp.max(n2[2:], axis=0, keepdims=True))

    x_copy(0).wait()
    for j in range(1, NQ):
        x_copy(j).start()
    cp_wq.wait()
    cp_wk.wait()
    cp_wv.wait()
    wT_ref[2 * DH:, :] = wq_ref[...].astype(f32).T.astype(bf16)
    n2 = project(0, layer_norm(0))
    for j in range(1, NQ):
        x_copy(j).wait()
    cp_w1.start()
    cp_w2.start()
    for j in range(1, NQ):
        n2 = tuple(jnp.maximum(a, b) for a, b in zip(n2, project(j, layer_norm(j))))

    k2 = jnp.max(n2[0])
    v2 = jnp.max(n2[1])
    q2 = jnp.max(n2[2]) * (QSCALE * QSCALE)
    fast = jnp.logical_and(
        q2 * k2 * 1.05 <= SCORE_BOUND * SCORE_BOUND,
        jnp.logical_and(v2 <= 2.0 ** 80, v2 >= 2.0 ** -60))
    never = q2 < -1.0

    def q_tile(t, ct):
        return unpack(qT_ref[pl.ds(pl.multiple_of(t * 8, 8), 8),
                             ct * 128:(ct + 1) * 128])

    def v_tile(c):
        jb, cc = divmod(c, TQ // TK)
        return unpack(vT_ref[jb, :, cc * TK:(cc + 1) * TK])

    def write_o(t, acc, l):
        lsum = jnp.sum(l, axis=0, keepdims=True)
        oT_ref[pl.ds(pl.multiple_of(t * DH, DH), DH), :] = (acc / lsum).astype(bf16)

    def q_rows(t, ct, first=False):
        rows = [jnp.broadcast_to(qf_ref[t, d:d + 1, ct * 128:(ct + 1) * 128],
                                 (16, 128)) for d in range(DH)]
        cuts = ([0, 1] if first else [0]) + list(range(UG, DH + 1, UG))
        return [(a, b, jnp.stack(rows[a:b])) for a, b in zip(cuts, cuts[1:])]

    def vpu_scores(kb, qb, trigger=None):
        sv = None
        for a, b, q in qb:
            pr = kb[a:b] * q
            if sv is not None:
                pr = jnp.concatenate([sv, pr], axis=0)
            if sv is None and trigger is not None:
                sv = jnp.where(never, trigger[None], pr)
            else:
                sv = jnp.sum(pr, axis=0, keepdims=True)
        return sv[0]

    def make_host(s0, ns, njobs):
        nunits = ns * NC * NCT
        per = -(-nunits // njobs)
        state = dict(done=0, job=0, qb=None)

        def hosted(res):
            for k in range(per):
                r0 = (k * TQ // per) // 16 * 16
                upto = (state["job"] * per + k + 1) * nunits // (njobs * per)
                while state["done"] < upto:
                    ks, rem = divmod(state["done"], NC * NCT)
                    ct, c = divmod(rem, NC)
                    if c == 0:
                        state["qb"] = q_rows(T - SP + s0 + ks, ct, first=True)
                    trig = res[r0:r0 + 16, 0:128]
                    if trig.shape[1] < 128:
                        trig = jnp.concatenate(
                            [trig, jnp.zeros((16, 128 - trig.shape[1]), f32)], axis=1)
                    sv_ref[s0 + ks, c, ct] = vpu_scores(
                        kbb_ref.at[c], state["qb"], trig)
                    state["done"] += 1
            state["job"] += 1
        return hosted

    def out_piece(k, hosted=None):
        r0, r1 = OUT_CUTS[k], OUT_CUTS[k + 1]
        j = r0 // TQ
        oT = lambda k0, k1: oT_ref[j * D + k0:j * D + k1, r0 - j * TQ:r1 - j * TQ]
        if hosted is None:
            a = lax.dot_general(oT(0, D), wo_ref[...], _TN, preferred_element_type=f32)
        else:
            a = None
            for kk in range(D // 128):
                p = lax.dot_general(oT(kk * 128, (kk + 1) * 128),
                                    wo_ref[kk * 128:(kk + 1) * 128, :], _TN,
                                    preferred_element_type=f32)
                hosted(p)
                a = p if a is None else a + p
        out_ref[r0:r1, :] = (xy_ref[r0:r1, :] + a).astype(bf16)
        out_copy(k).start()

    cp_w1.wait()
    cp_w2.wait()
    cp_wo.start()

    def ffn_body(j, carry):
        rows = pl.ds(pl.multiple_of(j * TQ, TQ), TQ)
        xn = xn_ref[rows, :]
        pos = sum(jnp.where(j == jq, 7 - POS_A[jq], 0) for jq in range(NQ))
        for cc in range(TQ // TK):
            c = j * (TQ // TK) + cc
            kf = unpack(km_ref[0, c, pl.ds(pl.multiple_of(pos * 8, 8), 8), :]
                        ).astype(f32)
            for d in range(DH):
                kba_ref[c, d] = jnp.broadcast_to(kf[:, d:d + 1], (16, 128))

        hosted = make_host(j * FS, FS, 2 * NFT)

        def up(n):
            h = lax.dot_general(xn, w1T_ref[n * 128:min((n + 1) * 128, F), :], _NT,
                                preferred_element_type=f32)
            hosted(h)
            hh = 0.5 * h
            return (hh * jnp.tanh(hh) + hh).astype(bf16)

        def down(g, n):
            y = jnp.dot(g, w2_ref[n * 128:min((n + 1) * 128, F), :],
                        preferred_element_type=f32)
            hosted(y)
            return y

        y = x_ref[rows, :].astype(f32)
        g = up(0)
        for n in range(NFT):
            gn = up(n + 1) if n + 1 < NFT else None
            y = y + down(g, n)
            g = gn
        xy_ref[rows, :] = y
        return carry

    lax.fori_loop(0, NQ, ffn_body, 0)

    def fast_phase(special_phase):
        def qk(t, n, special):
            out = []
            for ct in range(NCT):
                c = (n + 4 * ct) % NC
                kk = km_ref[2 if special else 1, c,
                            0:8 * len(_mxu_groups(c, special)), :]
                out.append(jnp.dot(unpack(kk), q_tile(t, ct),
                                   preferred_element_type=f32))
            return out

        def pv(n, s_m, qb, acc, l, s):
            ps = []
            for ct in range(NCT):
                c = (n + 4 * ct) % NC
                js = _mxu_groups(c, s is not None)
                parts, r0 = [], 0
                for j in range(8):
                    if j in js:
                        continue
                    r1 = 16 * len([jj for jj in js if jj < j])
                    if r1 > r0:
                        parts.append(s_m[ct][r0:r1])
                    r0 = r1
                    if j == POS_A[c // 4]:
                        parts.append(vpu_scores(kba_ref.at[c], qb[ct]))
                    else:
                        parts.append(sv_ref[s, c, ct])
                if r0 < 16 * len(js):
                    parts.append(s_m[ct][r0:])
                ps.append(jnp.concatenate(parts, axis=0))
            pw = jnp.exp2(jnp.concatenate(ps, axis=1))
            if l is not None:
                l = jnp.sum(jnp.concatenate([l, pw], axis=0).reshape(
                    TK // 8 + 1, 8, TQ), axis=0)
            else:
                l = jnp.sum(pw.reshape(TK // 8, 8, TQ), axis=0)
            pw = jnp.concatenate(
                [pw[j * 16:(j + 1) * 16] for j in reversed(range(8))], axis=0)
            for ct in range(NCT):
                o = jnp.dot(v_tile((n + 4 * ct) % NC),
                            pw[:, ct * 128:(ct + 1) * 128].astype(bf16),
                            preferred_element_type=f32)
                acc[ct] = o if acc[ct] is None else acc[ct] + o
            return acc, l

        def stash(s):
            for ct in range(NCT):
                sc_ref[ct] = s[ct]

        def make_body(t_base, special):
            def body(i, carry):
                nslots = UF * NC
                t0 = t_base + i * UF
                t_next = jnp.minimum(t0 + UF, T - 1)
                full = {0: [sc_ref[ct] for ct in range(NCT)]}
                for m in range(1, nslots + LAG):
                    if m < nslots:
                        full[m] = qk(t0 + m // NC, m % NC, special)
                    elif m == nslots:
                        stash(qk(t_next, 0, False))
                    n = m - LAG
                    if n >= 0:
                        u, c = divmod(n, NC)
                        if c == 0:
                            if u == 0:
                                acc, l = [None] * NCT, None
                            else:
                                acc, l = [a * 0.0 for a in acc], l * 0.0
                            qb = [q_rows(t0 + u, ct) for ct in range(NCT)]
                        s = i * UF + u if special and n > 0 else None
                        acc, l = pv(c, full.pop(n), qb, acc, l, s)
                        if c == NC - 1:
                            write_o(t0 + u, jnp.concatenate(acc, axis=1), l)
                return carry
            return body

        if not special_phase:
            stash(qk(0, 0, False))
            lax.fori_loop(0, NREG, make_body(0, False), 0)
        else:
            lax.fori_loop(0, SP // UF, make_body(T - SP, True), 0)

    pl.when(fast)(lambda: fast_phase(False))

    @pl.when(jnp.logical_not(fast))
    def _():
        def clear(c, carry):
            sbuf[c] = jnp.zeros((TK, TQ), f32)
            return carry

        lax.fori_loop(0, NC, clear, 0)

        def body(t, m_prev):
            ta = jnp.minimum(t, T - 1)

            def quad(jb, carry):
                m, acc, l = carry
                qh = unpack(qT_ref[pl.ds(pl.multiple_of(ta * 8, 8), 8), :])
                for cc in range(TQ // TK):
                    c = jb * (TQ // TK) + cc
                    p = jnp.exp2(sbuf[c] - m_prev)
                    acc = acc + jnp.dot(
                        unpack(vT_ref[jb, :, cc * TK:(cc + 1) * TK]),
                        p.astype(bf16), preferred_element_type=f32)
                    for r in reversed(range(TK // 8)):
                        l = l + p[r * 8:(r + 1) * 8, :]
                    s = jnp.dot(unpack(km_ref[0, c]), qh, preferred_element_type=f32)
                    sbuf[c] = s
                    m = jnp.maximum(m, jnp.max(s.reshape(TK // 8, 8, TQ), axis=0))
                return m, acc, l

            m, acc, l = lax.fori_loop(
                0, NQ, quad,
                (jnp.full((8, TQ), -jnp.inf, f32), jnp.zeros((DH, TQ), f32),
                 jnp.zeros((8, TQ), f32)))
            write_o(jnp.maximum(t - 1, 0), acc, l)
            return jnp.max(m, axis=0, keepdims=True)

        lax.fori_loop(0, T + 1, body, jnp.zeros((1, TQ), f32))

    cp_wo.wait()
    hosted = make_host(NQ * FS, OS, NEARLY * (D // 128))
    for k in range(NEARLY):
        out_piece(k, hosted)
    pl.when(fast)(lambda: fast_phase(True))
    for k in range(NEARLY, len(OUT_CUTS) - 1):
        out_piece(k)
    for k in range(len(OUT_CUTS) - 1):
        out_copy(k).wait()


@jax.jit
def pallas_parallel_sum__grouped_kv_mqa__dense_activation_silu__prompt_kernel(
    A_x: jax.Array,
    A_wq: jax.Array,
    A_wk: jax.Array,
    A_wv: jax.Array,
    A_wo: jax.Array,
    B_x: jax.Array,
    B_w1: jax.Array,
    B_w2: jax.Array,
):
    del B_x
    bf16 = jnp.bfloat16
    f32 = jnp.float32
    u32 = jnp.uint32
    any_spec = pl.BlockSpec(memory_space=pl.ANY)
    out = pl.pallas_call(
        _kernel,
        out_shape=jax.ShapeDtypeStruct((S, D), bf16),
        in_specs=[any_spec] * 7,
        out_specs=any_spec,
        scratch_shapes=[
            pltpu.VMEM((S, D), bf16),
            pltpu.VMEM((D, D), bf16),
            pltpu.VMEM((D, D), bf16),
            pltpu.VMEM((F, D), bf16),
            pltpu.VMEM((F, D), bf16),
            pltpu.VMEM((S, D), bf16),
            pltpu.VMEM((S, D), bf16),
            pltpu.VMEM((D + 2 * DH, D), bf16),
            pltpu.VMEM((3, NC, TK // 2, DH), u32),
            pltpu.VMEM((NQ, DH // 2, TQ), u32),
            pltpu.VMEM((NQ * D // 2, TQ), u32),
            pltpu.VMEM((T, DH, TQ), f32),
            pltpu.VMEM((NC, DH, 16, 128), f32),
            pltpu.VMEM((NC, DH, 16, 128), f32),
            pltpu.VMEM((NQ * D, TQ), bf16),
            pltpu.VMEM((S, D), f32),
            pltpu.VMEM((SP, NC, NCT, 16, 128), f32),
            pltpu.VMEM((NCT, TK - 16, 128), f32),
            pltpu.VMEM((NC, TK, TQ), f32),
            pltpu.SemaphoreType.DMA((NQ + 6 + len(OUT_CUTS) - 1,)),
        ],
        compiler_params=pltpu.CompilerParams(
            vmem_limit_bytes=100 * 1024 * 1024),
    )(A_x.reshape(S, D), A_wq, A_wk.T, A_wv.T, A_wo, B_w1.T, B_w2)
    return out.reshape(1, S, D)
```

```python
import math

import jax
import jax.numpy as jnp
from jax import lax
import jax.experimental.pallas as pl
import jax.experimental.pallas.tpu as pltpu

S = 2048
D = 512
H = 32
DH = 16
F = 1376
TQ = 512
NQ = S // TQ
NCT = TQ // 128
TK = 128
NC = S // TK
T = NQ * H
NFT = -(-F // 128)
EPS = 1e-5
QSCALE = (DH ** -0.5) * math.log2(math.e)
SCORE_BOUND = 60.0

UF = 8
NREG = 12
SP = T - UF * NREG
FS = 7
OS = SP - NQ * FS
NEARLY = 3
LAG = 2
UG = 4
POS_A = (0, 2, 4, 6)
POS_B = (4, 4, 0, 0)
OUT_CUTS = (0, 512, 1024, 1536, 1792, 1920, 2048)

_NT = (((1,), (1,)), ((), ()))
_TN = (((0,), (0,)), ((), ()))


def _mxu_groups(c, special):
    skip = (POS_A[c // 4], POS_B[c // 4]) if special else (POS_A[c // 4],)
    return [j for j in range(8) if j not in skip]


def _kernel(x_hbm, wq_hbm, wkT_hbm, wvT_hbm, wo_hbm, w1T_hbm, w2_hbm, o_hbm,
            x_ref, wq_ref, wo_ref, w1T_ref, w2_ref, out_ref,
            xn_ref, wT_ref, km_ref, vT_ref, qT_ref, qf_ref, kba_ref, kbb_ref,
            oT_ref, xy_ref, sv_ref, sc_ref, sbuf, sems):
    f32 = jnp.float32
    bf16 = jnp.bfloat16
    pack = lambda a: pltpu.bitcast(a, jnp.uint32)
    unpack = lambda a: pltpu.bitcast(a, bf16)

    def x_copy(j):
        rows = pl.ds(j * TQ, TQ)
        return pltpu.make_async_copy(x_hbm.at[rows], x_ref.at[rows], sems.at[j])

    cp_wq = pltpu.make_async_copy(wq_hbm, wq_ref, sems.at[NQ])
    cp_wk = pltpu.make_async_copy(wkT_hbm, wT_ref.at[pl.ds(0, DH)], sems.at[NQ + 1])
    cp_wv = pltpu.make_async_copy(wvT_hbm, wT_ref.at[pl.ds(DH, DH)], sems.at[NQ + 2])
    cp_w1 = pltpu.make_async_copy(w1T_hbm, w1T_ref, sems.at[NQ + 3])
    cp_w2 = pltpu.make_async_copy(w2_hbm, w2_ref, sems.at[NQ + 4])
    cp_wo = pltpu.make_async_copy(wo_hbm, wo_ref, sems.at[NQ + 5])

    def out_copy(k):
        rows = pl.ds(OUT_CUTS[k], OUT_CUTS[k + 1] - OUT_CUTS[k])
        return pltpu.make_async_copy(out_ref.at[rows], o_hbm.at[rows],
                                     sems.at[NQ + 6 + k])

    x_copy(0).start()
    cp_wq.start()
    cp_wk.start()
    cp_wv.start()

    def layer_norm(j):
        rows = slice(j * TQ, (j + 1) * TQ)
        x = x_ref[rows, :].astype(f32)
        mu = jnp.mean(x, axis=-1, keepdims=True)
        xc = x - mu
        var = jnp.mean(xc * xc, axis=-1, keepdims=True)
        xn = (xc * lax.rsqrt(var + EPS)).astype(bf16)
        xn_ref[rows, :] = xn
        return xn

    def project(j, xn):
        r = lax.dot_general(wT_ref[...], xn, _NT, preferred_element_type=f32)
        kr = r[0:DH].T.astype(bf16)
        kp = pack(kr)
        kf = kr.astype(f32)
        for cc in range(TQ // TK):
            c = j * (TQ // TK) + cc
            km_ref[0, c] = kp[cc * 64:(cc + 1) * 64]
            for v, special in ((1, False), (2, True)):
                js = _mxu_groups(c, special)
                km_ref[v, c, 0:8 * len(js), :] = jnp.concatenate(
                    [kp[(cc * 8 + 7 - jj) * 8:(cc * 8 + 8 - jj) * 8] for jj in js],
                    axis=0)
            k0 = (cc * 8 + 7 - POS_B[j]) * 16
            for d in range(DH):
                kbb_ref[c, d] = jnp.broadcast_to(kf[k0:k0 + 16, d:d + 1], (16, 128))
        vT_ref[j] = pack(r[DH:2 * DH].astype(bf16))
        q = (r[2 * DH:] * QSCALE).astype(bf16)
        qT_ref[j * (D // 2):(j + 1) * (D // 2), :] = pack(q)
        qf_ref[j * H:(j + 1) * H] = q.astype(f32).reshape(H, DH, TQ)
        n2 = jnp.sum((r * r).reshape(H + 2, DH, TQ), axis=1)
        return (n2[0:1], n2[1:2], jnp.max(n2[2:], axis=0, keepdims=True))

    x_copy(0).wait()
    for j in range(1, NQ):
        x_copy(j).start()
    cp_wq.wait()
    cp_wk.wait()
    cp_wv.wait()
    wT_ref[2 * DH:, :] = wq_ref[...].astype(f32).T.astype(bf16)
    n2 = project(0, layer_norm(0))
    for j in range(1, NQ):
        x_copy(j).wait()
    cp_w1.start()
    cp_w2.start()
    for j in range(1, NQ):
        n2 = tuple(jnp.maximum(a, b) for a, b in zip(n2, project(j, layer_norm(j))))

    k2 = jnp.max(n2[0])
    v2 = jnp.max(n2[1])
    q2 = jnp.max(n2[2]) * (QSCALE * QSCALE)
    fast = jnp.logical_and(
        q2 * k2 * 1.05 <= SCORE_BOUND * SCORE_BOUND,
        jnp.logical_and(v2 <= 2.0 ** 80, v2 >= 2.0 ** -60))
    never = q2 < -1.0

    def q_tile(t, ct):
        return unpack(qT_ref[pl.ds(pl.multiple_of(t * 8, 8), 8),
                             ct * 128:(ct + 1) * 128])

    def v_tile(c):
        jb, cc = divmod(c, TQ // TK)
        return unpack(vT_ref[jb, :, cc * TK:(cc + 1) * TK])

    def write_o(t, acc, l):
        lsum = jnp.sum(l, axis=0, keepdims=True)
        oT_ref[pl.ds(pl.multiple_of(t * DH, DH), DH), :] = (acc / lsum).astype(bf16)

    def q_rows(t, ct, first=False):
        rows = [jnp.broadcast_to(qf_ref[t, d:d + 1, ct * 128:(ct + 1) * 128],
                                 (16, 128)) for d in range(DH)]
        cuts = ([0, 1] if first else [0]) + list(range(UG, DH + 1, UG))
        return [(a, b, jnp.stack(rows[a:b])) for a, b in zip(cuts, cuts[1:])]

    def vpu_scores(kb, qb, trigger=None):
        sv = None
        for a, b, q in qb:
            pr = kb[a:b] * q
            if sv is not None:
                pr = jnp.concatenate([sv, pr], axis=0)
            if sv is None and trigger is not None:
                sv = jnp.where(never, trigger[None], pr)
            else:
                sv = jnp.sum(pr, axis=0, keepdims=True)
        return sv[0]

    def make_host(s0, ns, njobs):
        nunits = ns * NC * NCT
        per = -(-nunits // njobs)
        state = dict(done=0, job=0, qb=None)

        def hosted(res):
            for k in range(per):
                r0 = (k * TQ // per) // 16 * 16
                upto = (state["job"] * per + k + 1) * nunits // (njobs * per)
                while state["done"] < upto:
                    ks, rem = divmod(state["done"], NC * NCT)
                    ct, c = divmod(rem, NC)
                    if c == 0:
                        state["qb"] = q_rows(T - SP + s0 + ks, ct, first=True)
                    trig = res[r0:r0 + 16, 0:128]
                    if trig.shape[1] < 128:
                        trig = jnp.concatenate(
                            [trig, jnp.zeros((16, 128 - trig.shape[1]), f32)], axis=1)
                    sv_ref[s0 + ks, c, ct] = vpu_scores(
                        kbb_ref.at[c], state["qb"], trig)
                    state["done"] += 1
            state["job"] += 1
        return hosted

    def out_piece(k, hosted=None):
        r0, r1 = OUT_CUTS[k], OUT_CUTS[k + 1]
        j = r0 // TQ
        oT = lambda k0, k1: oT_ref[j * D + k0:j * D + k1, r0 - j * TQ:r1 - j * TQ]
        if hosted is None:
            a = lax.dot_general(oT(0, D), wo_ref[...], _TN, preferred_element_type=f32)
        else:
            a = None
            for kk in range(D // 128):
                p = lax.dot_general(oT(kk * 128, (kk + 1) * 128),
                                    wo_ref[kk * 128:(kk + 1) * 128, :], _TN,
                                    preferred_element_type=f32)
                hosted(p)
                a = p if a is None else a + p
        out_ref[r0:r1, :] = (xy_ref[r0:r1, :] + a).astype(bf16)
        out_copy(k).start()

    cp_w1.wait()
    cp_w2.wait()
    cp_wo.start()

    def ffn_body(j, carry):
        rows = pl.ds(pl.multiple_of(j * TQ, TQ), TQ)
        xn = xn_ref[rows, :]
        pos = sum(jnp.where(j == jq, 7 - POS_A[jq], 0) for jq in range(NQ))
        for cc in range(TQ // TK):
            c = j * (TQ // TK) + cc
            kf = unpack(km_ref[0, c, pl.ds(pl.multiple_of(pos * 8, 8), 8), :]
                        ).astype(f32)
            for d in range(DH):
                kba_ref[c, d] = jnp.broadcast_to(kf[:, d:d + 1], (16, 128))

        hosted = make_host(j * FS, FS, 2 * NFT)

        def up(n):
            h = lax.dot_general(xn, w1T_ref[n * 128:min((n + 1) * 128, F), :], _NT,
                                preferred_element_type=f32)
            hosted(h)
            hh = 0.5 * h
            return (hh * jnp.tanh(hh) + hh).astype(bf16)

        def down(g, n):
            y = jnp.dot(g, w2_ref[n * 128:min((n + 1) * 128, F), :],
                        preferred_element_type=f32)
            hosted(y)
            return y

        y = x_ref[rows, :].astype(f32)
        g = up(0)
        for n in range(NFT):
            gn = up(n + 1) if n + 1 < NFT else None
            y = y + down(g, n)
            g = gn
        xy_ref[rows, :] = y
        return carry

    lax.fori_loop(0, NQ, ffn_body, 0)

    def qk(t, n, special):
        out = []
        for ct in range(NCT):
            c = (n + 4 * ct) % NC
            kk = km_ref[2 if special else 1, c,
                        0:8 * len(_mxu_groups(c, special)), :]
            out.append(jnp.dot(unpack(kk), q_tile(t, ct),
                               preferred_element_type=f32))
        return out

    def stash(s):
        for ct in range(NCT):
            sc_ref[ct, 0:s[ct].shape[0], :] = s[ct]

    def fast_phase(special_phase):
        def pv(n, s_m, qb, acc, l, s):
            ps = []
            for ct in range(NCT):
                c = (n + 4 * ct) % NC
                js = _mxu_groups(c, s is not None)
                parts, r0 = [], 0
                for j in range(8):
                    if j in js:
                        continue
                    r1 = 16 * len([jj for jj in js if jj < j])
                    if r1 > r0:
                        parts.append(s_m[ct][r0:r1])
                    r0 = r1
                    if j == POS_A[c // 4]:
                        parts.append(vpu_scores(kba_ref.at[c], qb[ct]))
                    else:
                        parts.append(sv_ref[s, c, ct])
                if r0 < 16 * len(js):
                    parts.append(s_m[ct][r0:])
                ps.append(jnp.concatenate(parts, axis=0))
            pw = jnp.exp2(jnp.concatenate(ps, axis=1))
            if l is not None:
                l = jnp.sum(jnp.concatenate([l, pw], axis=0).reshape(
                    TK // 8 + 1, 8, TQ), axis=0)
            else:
                l = jnp.sum(pw.reshape(TK // 8, 8, TQ), axis=0)
            pw = jnp.concatenate(
                [pw[j * 16:(j + 1) * 16] for j in reversed(range(8))], axis=0)
            for ct in range(NCT):
                o = jnp.dot(v_tile((n + 4 * ct) % NC),
                            pw[:, ct * 128:(ct + 1) * 128].astype(bf16),
                            preferred_element_type=f32)
                acc[ct] = o if acc[ct] is None else acc[ct] + o
            return acc, l

        def make_body(t_base, special):
            def body(i, carry):
                nslots = UF * NC
                t0 = t_base + i * UF
                t_next = jnp.minimum(t0 + UF, T - 1)
                nrows = 16 * len(_mxu_groups(0, special))
                full = {0: [sc_ref[ct, 0:nrows, :] for ct in range(NCT)]}
                for m in range(1, nslots + LAG):
                    if m < nslots:
                        full[m] = qk(t0 + m // NC, m % NC, special)
                    elif m == nslots:
                        stash(qk(t_next, 0, special))
                    n = m - LAG
                    if n >= 0:
                        u, c = divmod(n, NC)
                        if c == 0:
                            if u == 0:
                                acc, l = [None] * NCT, None
                            else:
                                acc, l = [a * 0.0 for a in acc], l * 0.0
                            qb = [q_rows(t0 + u, ct) for ct in range(NCT)]
                        s = i * UF + u if special else None
                        acc, l = pv(c, full.pop(n), qb, acc, l, s)
                        if c == NC - 1:
                            write_o(t0 + u, jnp.concatenate(acc, axis=1), l)
                return carry
            return body

        if not special_phase:
            stash(qk(0, 0, False))
            lax.fori_loop(0, NREG, make_body(0, False), 0)
        else:
            lax.fori_loop(0, SP // UF, make_body(T - SP, True), 0)

    def safe_phase(t_lo, t_hi):
        def clear(c, carry):
            sbuf[c] = jnp.zeros((TK, TQ), f32)
            return carry

        lax.fori_loop(0, NC, clear, 0)

        def body(t, m_prev):
            ta = jnp.minimum(t, t_hi - 1)

            def quad(jb, carry):
                m, acc, l = carry
                qh = unpack(qT_ref[pl.ds(pl.multiple_of(ta * 8, 8), 8), :])
                for cc in range(TQ // TK):
                    c = jb * (TQ // TK) + cc
                    p = jnp.exp2(sbuf[c] - m_prev)
                    acc = acc + jnp.dot(
                        unpack(vT_ref[jb, :, cc * TK:(cc + 1) * TK]),
                        p.astype(bf16), preferred_element_type=f32)
                    for r in reversed(range(TK // 8)):
                        l = l + p[r * 8:(r + 1) * 8, :]
                    s = jnp.dot(unpack(km_ref[0, c]), qh, preferred_element_type=f32)
                    sbuf[c] = s
                    m = jnp.maximum(m, jnp.max(s.reshape(TK // 8, 8, TQ), axis=0))
                return m, acc, l

            m, acc, l = lax.fori_loop(
                0, NQ, quad,
                (jnp.full((8, TQ), -jnp.inf, f32), jnp.zeros((DH, TQ), f32),
                 jnp.zeros((8, TQ), f32)))
            write_o(jnp.maximum(t - 1, t_lo), acc, l)
            return jnp.max(m, axis=0, keepdims=True)

        lax.fori_loop(t_lo, t_hi + 1, body, jnp.zeros((1, TQ), f32))

    lax.cond(fast, lambda: fast_phase(False), lambda: safe_phase(0, T - SP))

    cp_wo.wait()
    hosted = make_host(NQ * FS, OS, NEARLY * (D // 128))
    for k in range(NEARLY):
        out_piece(k, hosted)
    stash(qk(T - SP, 0, True))
    lax.cond(fast, lambda: fast_phase(True), lambda: safe_phase(T - SP, T))
    for k in range(NEARLY, len(OUT_CUTS) - 1):
        out_piece(k)
    for k in range(len(OUT_CUTS) - 1):
        out_copy(k).wait()


@jax.jit
def pallas_parallel_sum__grouped_kv_mqa__dense_activation_silu__prompt_kernel(
    A_x: jax.Array,
    A_wq: jax.Array,
    A_wk: jax.Array,
    A_wv: jax.Array,
    A_wo: jax.Array,
    B_x: jax.Array,
    B_w1: jax.Array,
    B_w2: jax.Array,
):
    del B_x
    bf16 = jnp.bfloat16
    f32 = jnp.float32
    u32 = jnp.uint32
    any_spec = pl.BlockSpec(memory_space=pl.ANY)
    out = pl.pallas_call(
        _kernel,
        out_shape=jax.ShapeDtypeStruct((S, D), bf16),
        in_specs=[any_spec] * 7,
        out_specs=any_spec,
        scratch_shapes=[
            pltpu.VMEM((S, D), bf16),
            pltpu.VMEM((D, D), bf16),
            pltpu.VMEM((D, D), bf16),
            pltpu.VMEM((F, D), bf16),
            pltpu.VMEM((F, D), bf16),
            pltpu.VMEM((S, D), bf16),
            pltpu.VMEM((S, D), bf16),
            pltpu.VMEM((D + 2 * DH, D), bf16),
            pltpu.VMEM((3, NC, TK // 2, DH), u32),
            pltpu.VMEM((NQ, DH // 2, TQ), u32),
            pltpu.VMEM((NQ * D // 2, TQ), u32),
            pltpu.VMEM((T, DH, TQ), f32),
            pltpu.VMEM((NC, DH, 16, 128), f32),
            pltpu.VMEM((NC, DH, 16, 128), f32),
            pltpu.VMEM((NQ * D, TQ), bf16),
            pltpu.VMEM((S, D), f32),
            pltpu.VMEM((SP, NC, NCT, 16, 128), f32),
            pltpu.VMEM((NCT, TK - 16, 128), f32),
            pltpu.VMEM((NC, TK, TQ), f32),
            pltpu.SemaphoreType.DMA((NQ + 6 + len(OUT_CUTS) - 1,)),
        ],
        compiler_params=pltpu.CompilerParams(
            vmem_limit_bytes=100 * 1024 * 1024),
    )(A_x.reshape(S, D), A_wq, A_wk.T, A_wv.T, A_wo, B_w1.T, B_w2)
    return out.reshape(1, S, D)
```
